```python
import jax
import jax.numpy as jnp

def _softmax(x, axis=-1):
    return jax.nn.softmax(x, axis=axis)
def _gelu(x):
    return jax.nn.gelu(x, approximate=True)
def _silu(x):
    return jax.nn.silu(x)
def _sigmoid(x):
    return jax.nn.sigmoid(x)
def _layernorm(x, axis=-1, eps=1e-5):
    m = jnp.mean(x, axis=axis, keepdims=True)
    v = jnp.var(x, axis=axis, keepdims=True)
    return (x - m) / jnp.sqrt(v + eps)
def _scatter_add(tgt, idx, src, axis=0):
    return tgt.at[idx].add(src)
def _segment_sum(src, seg, n):
    return jax.ops.segment_sum(src, seg, n)
class _Rng:
    def __init__(self, key):
        self._k = key
    def _next(self):
        self._k, sub = jax.random.split(self._k)
        return sub
    def normal(self, shape):
        return jax.random.normal(self._next(), shape, dtype=jnp.bfloat16)
    def randint(self, lo, hi, shape):
        return jax.random.randint(self._next(), shape, lo, hi, dtype=jnp.int32)
    def uniform(self, shape, lo=0.0, hi=1.0):
        return jax.random.uniform(self._next(), shape, jnp.bfloat16, lo, hi)
    def permutation(self, n):
        return jax.random.permutation(self._next(), n)


kernel_name = 'sequential_preLN__sliding_block_cached__moe_arch_mod__decode'

def setup_inputs():
    _rng = _Rng(jax.random.key(int.from_bytes(__import__("os").urandom(4), "little")))
    _w = (lambda a: (lambda t: t.astype(jnp.bfloat16) if jnp.issubdtype(t.dtype, jnp.floating) else t)(jnp.asarray(a)))
    def _A_setup():
        B, Sq, D = 1, 1, 640
        Hq, Hkv, Sk, Dh = 32, 32, 32768, 192
        assert Hq % Hkv == 0, (Hq, Hkv)
        return {
            "x": _w((lambda *s: _rng.normal(s) * 0.05)(B, Sq, D)),
            "k_cache": _w((lambda *s: _rng.normal(s) * 0.05)(B, Hkv, Sk, Dh)),
            "v_cache": _w((lambda *s: _rng.normal(s) * 0.05)(B, Hkv, Sk, Dh)),
            "wq": _w((lambda *s: _rng.normal(s) * 0.05)(D, Hq * Dh) * (D ** -0.5)),
            "wo": _w((lambda *s: _rng.normal(s) * 0.05)(Hq * Dh, D) * ((Hq * Dh) ** -0.5)),
        }
    _A_in = _A_setup()

    def _B_setup():
        B, S, D, F, C = 1, 1, 640, 1536, 1
        return {
            "x": _w((lambda *s: _rng.normal(s) * 0.05)(B, S, D)),
            "w_r": _w((lambda *s: _rng.normal(s) * 0.05)(D)),
            "w_gate": _w((lambda *s: _rng.normal(s) * 0.05)(D, F)),
            "w_up": _w((lambda *s: _rng.normal(s) * 0.05)(D, F)),
            "w_down": _w((lambda *s: _rng.normal(s) * 0.05)(F, D)),
        }
    _B_in = _B_setup()

    return {
        "A_x": _A_in["x"],
        "A_k_cache": _A_in["k_cache"],
        "A_v_cache": _A_in["v_cache"],
        "A_wq": _A_in["wq"],
        "A_wo": _A_in["wo"],
        "B_x": _B_in["x"],
        "B_w_r": _B_in["w_r"],
        "B_w_gate": _B_in["w_gate"],
        "B_w_up": _B_in["w_up"],
        "B_w_down": _B_in["w_down"],
    }

def reference(A_x, A_k_cache, A_v_cache, A_wq, A_wo, B_x, B_w_r, B_w_gate, B_w_up, B_w_down):
    def _A_ref(x, k_cache, v_cache, wq, wo):
        B, Sq, D = x.shape
        Hq, Dh = 32, 192
        Hkv, Sk = k_cache.shape[1], k_cache.shape[2]
        W = min(4096, max(256, Sk // 4))
        rep = Hq // Hkv
        q = (lambda x, *d: x.transpose(*d))((x @ wq).reshape(B, Sq, Hq, Dh), 0, 2, 1, 3)
        k = jnp.repeat(k_cache[:, :, Sk - W:, :], rep, axis=1)
        v = jnp.repeat(v_cache[:, :, Sk - W:, :], rep, axis=1)
        scores = jnp.einsum("bhqd,bhkd->bhqk", q, k) * (Dh ** -0.5)
        p = _softmax(scores, axis=-1)
        o = jnp.einsum("bhqk,bhkd->bhqd", p, v)
        return (lambda x, *d: x.transpose(*d))(o, 0, 2, 1, 3).reshape(B, Sq, Hq * Dh) @ wo

    def _B_ref(x, w_r, w_gate, w_up, w_down):
        B, S, D = x.shape
        C = 1
        r = x @ w_r
        idx = jnp.argsort(-r, axis=-1)[:, :C]
        idx_e = jnp.repeat(idx.reshape(B, C, 1), D, axis=2)
        x_sel = jnp.take_along_axis(x, idx_e, axis=1)
        g = _silu(x_sel @ w_gate)
        u = x_sel @ w_up
        y = (g * u) @ w_down
        r_sel = _sigmoid(jnp.take_along_axis(r, idx, axis=1))
        y = y * r_sel.reshape(B, C, 1)
        b_off = (jnp.arange(B) * S).reshape(B, 1)
        flat_idx = (idx + b_off).reshape(B * C)
        zero = (x * 0.0).reshape(B * S, D)
        upd = _scatter_add(zero, flat_idx, y.reshape(B * C, D), axis=0)
        return x + upd.reshape(B, S, D)

    x = A_x
    h = x + _A_ref(_layernorm(x, axis=-1), A_k_cache, A_v_cache, A_wq, A_wo)
    h2 = h + _B_ref(_layernorm(h, axis=-1), B_w_r, B_w_gate, B_w_up, B_w_down)
    return h2
```

```python
import jax
import jax.numpy as jnp
from jax import lax
import jax.experimental.pallas as pl
import jax.experimental.pallas.tpu as pltpu

NBUF = 4
DOWN_CHUNKS = 4
EPS = 1e-5


def _layernorm(x):
    m = jnp.mean(x, axis=-1, keepdims=True)
    d = x - m
    v = jnp.mean(d * d, axis=-1, keepdims=True)
    return d / jnp.sqrt(v + EPS)


def _kernel(x_hbm, kt_hbm, vt_hbm, wq_hbm, wo_hbm, wr_hbm, wg_hbm, wu_hbm, wd_hbm,
            o_ref,
            x_s, wr_s, wq_s, wo_s, wg_s, wu_s, wd_s, k_s, v_s, q_s, p_s, acc_s,
            sem_w, sem_d, sem_k, sem_v):
    _, H, Dh, Sk = kt_hbm.shape
    W = k_s.shape[-1]
    D = x_hbm.shape[-1]
    F = wg_hbm.shape[-1]
    FC = F // DOWN_CHUNKS
    f32, bf16 = jnp.float32, jnp.bfloat16

    def k_cp(h):
        return pltpu.make_async_copy(
            kt_hbm.at[0, h, :, pl.ds(Sk - W, W)], k_s.at[h % NBUF], sem_k.at[h % NBUF])

    def v_cp(h):
        return pltpu.make_async_copy(
            vt_hbm.at[0, h, :, pl.ds(Sk - W, W)], v_s.at[h % NBUF], sem_v.at[h % NBUF])

    wq_cp = pltpu.make_async_copy(wq_hbm, wq_s, sem_w.at[0])
    x_cp = pltpu.make_async_copy(x_hbm, x_s, sem_w.at[1])
    wo_cp = pltpu.make_async_copy(wo_hbm, wo_s, sem_w.at[2])
    wg_cp = pltpu.make_async_copy(wg_hbm, wg_s, sem_w.at[3])
    wu_cp = pltpu.make_async_copy(wu_hbm, wu_s, sem_w.at[4])
    wr_cp = pltpu.make_async_copy(wr_hbm, wr_s, sem_w.at[5])
    wd_cp = [pltpu.make_async_copy(wd_hbm.at[pl.ds(c * FC, FC)], wd_s.at[pl.ds(c * FC, FC)],
                                   sem_d.at[c]) for c in range(DOWN_CHUNKS)]

    wq_cp.start()
    x_cp.start()
    wr_cp.start()
    wo_cp.start()
    for h in range(NBUF):
        k_cp(h).start()
        v_cp(h).start()

    x_cp.wait()
    x = x_s[0].astype(f32)
    xn = jnp.broadcast_to(_layernorm(x), (8, D)).astype(bf16)
    wq_cp.wait()
    QC = 2 * Dh
    for c in range(H // 2):
        q2 = jnp.dot(xn, wq_s[:, c * QC:(c + 1) * QC], preferred_element_type=f32)
        q_s[2 * c] = q2[:, :Dh]
        q_s[2 * c + 1] = q2[:, Dh:]
    acc_s[...] = jnp.zeros_like(acc_s)
    wo_cp.wait()

    scale = Dh ** -0.5

    def head(h, carry):
        slot = h % NBUF
        k_cp(h).wait()
        s = jnp.dot(q_s[h].astype(bf16), k_s[slot], preferred_element_type=f32) * scale

        @pl.when(h + NBUF < H)
        def _():
            k_cp(h + NBUF).start()

        @pl.when(h + NBUF == H)
        def _():
            wg_cp.start()
            wu_cp.start()

        m = jnp.max(s, axis=-1, keepdims=True)
        e = jnp.exp(s - m)
        l = jnp.sum(e, axis=-1, keepdims=True)
        p_s[...] = e
        inv = 1.0 / l
        v_cp(h).wait()
        row0 = pl.multiple_of(h * Dh, 64)
        acc = acc_s[...]
        for r in range(Dh // 16):
            a0 = jnp.zeros((8, 128), f32)
            a1 = jnp.zeros((8, 128), f32)
            for j in range(W // 128):
                vv = v_s[slot, r * 16:(r + 1) * 16, j * 128:(j + 1) * 128].astype(f32)
                pp = p_s[:, j * 128:(j + 1) * 128]
                a0 = a0 + vv[:8] * pp
                a1 = a1 + vv[8:] * pp
            o0 = jnp.sum(a0, axis=-1, keepdims=True) * inv
            o1 = jnp.sum(a1, axis=-1, keepdims=True) * inv
            ww = wo_s[pl.ds(row0 + r * 16, 16), :].astype(f32)
            acc = acc + ww[:8] * o0 + ww[8:] * o1
        acc_s[...] = acc

        @pl.when(h + NBUF < H)
        def _():
            v_cp(h + NBUF).start()

        @pl.when(h + NBUF == H)
        def _():
            for c in wd_cp:
                c.start()
        return carry

    lax.fori_loop(0, H, head, 0)

    hres = x + jnp.sum(acc_s[...], axis=0, keepdims=True)
    hn = _layernorm(hres)
    wr_cp.wait()
    wr = wr_s[...].astype(f32).reshape(1, D)
    gate = jax.nn.sigmoid(jnp.sum(hn * wr, axis=-1, keepdims=True))
    hb = jnp.broadcast_to(hn, (8, D)).astype(bf16)
    wg_cp.wait()
    g = jnp.dot(hb, wg_s[...], preferred_element_type=f32)
    wu_cp.wait()
    u = jnp.dot(hb, wu_s[...], preferred_element_type=f32)
    gu = (g * jax.nn.sigmoid(g) * u).astype(bf16)
    y = jnp.zeros((8, D), f32)
    for c in range(DOWN_CHUNKS):
        wd_cp[c].wait()
        y = y + jnp.dot(gu[:, c * FC:(c + 1) * FC], wd_s[c * FC:(c + 1) * FC, :],
                        preferred_element_type=f32)
    out = hres + (hn + y[:1] * gate)
    o_ref[0] = out.astype(o_ref.dtype)


@jax.jit
def pallas_sequential_preLN__sliding_block_cached__moe_arch_mod__decode_kernel(
    A_x: jax.Array,
    A_k_cache: jax.Array,
    A_v_cache: jax.Array,
    A_wq: jax.Array,
    A_wo: jax.Array,
    B_x: jax.Array,
    B_w_r: jax.Array,
    B_w_gate: jax.Array,
    B_w_up: jax.Array,
    B_w_down: jax.Array,
):
    del B_x
    _, H, Sk, Dh = A_k_cache.shape
    D = A_x.shape[-1]
    W = min(4096, max(256, Sk // 4))
    kt = jnp.transpose(A_k_cache, (0, 1, 3, 2))
    vt = jnp.transpose(A_v_cache, (0, 1, 3, 2))
    like = lambda a: pltpu.VMEM(a.shape, a.dtype)
    return pl.pallas_call(
        _kernel,
        out_shape=jax.ShapeDtypeStruct(A_x.shape, A_x.dtype),
        in_specs=[pl.BlockSpec(memory_space=pl.ANY)] * 9,
        scratch_shapes=[
            like(A_x), like(B_w_r), like(A_wq), like(A_wo),
            like(B_w_gate), like(B_w_up), like(B_w_down),
            pltpu.VMEM((NBUF, Dh, W), A_k_cache.dtype),
            pltpu.VMEM((NBUF, Dh, W), A_v_cache.dtype),
            pltpu.VMEM((H, 8, Dh), jnp.float32),
            pltpu.VMEM((8, W), jnp.float32),
            pltpu.VMEM((8, D), jnp.float32),
            pltpu.SemaphoreType.DMA((6,)),
            pltpu.SemaphoreType.DMA((DOWN_CHUNKS,)),
            pltpu.SemaphoreType.DMA((NBUF,)),
            pltpu.SemaphoreType.DMA((NBUF,)),
        ],
        compiler_params=pltpu.CompilerParams(vmem_limit_bytes=100 * 2**20),
    )(A_x, kt, vt, A_wq, A_wo, B_w_r, B_w_gate, B_w_up, B_w_down)
```

```python
import functools
import jax
import jax.numpy as jnp
from jax import lax
import jax.experimental.pallas as pl
import jax.experimental.pallas.tpu as pltpu

CR, CC = 32, 512
NBUF = 4
DOWN_CHUNKS = 4
EPS = 1e-5


def _layernorm(x):
    m = jnp.mean(x, axis=-1, keepdims=True)
    d = x - m
    v = jnp.mean(d * d, axis=-1, keepdims=True)
    return d / jnp.sqrt(v + EPS)


def _kernel(x_hbm, kt_hbm, vt_hbm, wq_hbm, wo_hbm, wr_hbm, wg_hbm, wu_hbm, wd_hbm,
            o_ref,
            x_s, wr_s, wq_s, wo_s, wg_s, wu_s, wd_s, k_s, v_s, q_s, p_s, acc_s,
            sem_w, sem_d, sem_k, sem_v):
    _, H, Dh, Sk = kt_hbm.shape
    W = k_s.shape[-1]
    D = x_hbm.shape[-1]
    F = wg_hbm.shape[-1]
    FC = F // DOWN_CHUNKS
    f32, bf16 = jnp.float32, jnp.bfloat16

    def piece(src, dst, sem, r, c, nc, prio):
        idx = (pl.ds(r, CR), pl.ds(c, nc))
        pltpu.make_async_copy(src.at[idx], dst.at[idx], sem).start(priority=prio)

    def done(dst, sem):
        pltpu.make_async_copy(dst, dst, sem).wait()

    kv_pieces = [(r, c) for r in range(0, Dh, CR) for c in range(0, W, CC)]

    def kv_start(h, pieces):
        sl = h % NBUF
        ks = kt_hbm.at[0, h, :, pl.ds(Sk - W, W)]
        vs = vt_hbm.at[0, h, :, pl.ds(Sk - W, W)]
        for r, c in pieces:
            piece(ks, k_s.at[sl], sem_k.at[sl], r, c, CC, 0)
            piece(vs, v_s.at[sl], sem_v.at[sl], r, c, CC, 1)

    def wide_start(src, dst, sem):
        def body(i, _):
            r = pl.multiple_of(i * CR, CR)
            for n, c in enumerate(range(0, src.shape[1], CC)):
                piece(src, dst, sem, r, c, CC, n % 2)
        lax.fori_loop(0, src.shape[0] // CR, body, None)

    def tall_start(src, dst, sem, r0, n):
        def body(i, _):
            for t in range(2):
                piece(src, dst, sem, pl.multiple_of(r0 + (2 * i + t) * CR, CR), 0, D, t)
        lax.fori_loop(0, n // CR // 2, body, None)

    def ffn_start():
        def body(i, _):
            r = pl.multiple_of(i * CR, CR)
            for c in range(0, F, CC):
                piece(wg_hbm, wg_s, sem_w.at[3], r, c, CC, 0)
                piece(wu_hbm, wu_s, sem_w.at[4], r, c, CC, 1)
        lax.fori_loop(0, D // CR, body, None)

    x_cp = pltpu.make_async_copy(x_hbm, x_s, sem_w.at[1])
    wr_cp = pltpu.make_async_copy(wr_hbm, wr_s, sem_w.at[5])

    x_cp.start()
    wr_cp.start(priority=1)
    wide_start(wq_hbm, wq_s, sem_w.at[0])
    tall_start(wo_hbm, wo_s, sem_w.at[2], 0, H * Dh)

    x_cp.wait()
    x = x_s[0].astype(f32)
    xn = jnp.broadcast_to(_layernorm(x), (8, D)).astype(bf16)
    done(wq_s, sem_w.at[0])
    QC = 2 * Dh
    for c in range(H // 2):
        if c < (NBUF - 1) * 4:
            kv_start(c // 4, kv_pieces[(c % 4) * 12:(c % 4 + 1) * 12])
        q2 = jnp.dot(xn, wq_s[:, c * QC:(c + 1) * QC], preferred_element_type=f32)
        q_s[2 * c] = q2[:, :Dh]
        q_s[2 * c + 1] = q2[:, Dh:]
    acc_s[...] = jnp.zeros_like(acc_s)
    done(wo_s, sem_w.at[2])

    scale = Dh ** -0.5

    def head(start, h, carry):
        slot = h % NBUF
        done(k_s.at[slot], sem_k.at[slot])
        s = jnp.dot(q_s[h].astype(bf16), k_s[slot], preferred_element_type=f32) * scale
        m = jnp.max(s, axis=-1, keepdims=True)
        e = jnp.exp(s - m)
        l = jnp.sum(e, axis=-1, keepdims=True)
        p_s[...] = e
        inv = 1.0 / l
        done(v_s.at[slot], sem_v.at[slot])
        row0 = pl.multiple_of(h * Dh, 64)
        acc = acc_s[...]
        for r in range(Dh // 16):
            start(h, r)
            a0 = jnp.zeros((8, 128), f32)
            a1 = jnp.zeros((8, 128), f32)
            for j in range(W // 128):
                vv = v_s[slot, r * 16:(r + 1) * 16, j * 128:(j + 1) * 128].astype(f32)
                pp = p_s[:, j * 128:(j + 1) * 128]
                a0 = a0 + vv[:8] * pp
                a1 = a1 + vv[8:] * pp
            o0 = jnp.sum(a0, axis=-1, keepdims=True) * inv
            o1 = jnp.sum(a1, axis=-1, keepdims=True) * inv
            ww = wo_s[pl.ds(row0 + r * 16, 16), :].astype(f32)
            acc = acc + ww[:8] * o0 + ww[8:] * o1
        acc_s[...] = acc
        return carry

    NL = NBUF - 1
    PR = len(kv_pieces) // (Dh // 16)
    lax.fori_loop(0, H - NL, functools.partial(
        head, lambda h, r: kv_start(h + NL, kv_pieces[r * PR:(r + 1) * PR])), 0)

    def tail_start(h, r):
        if r == 0:
            pl.when(h == H - NL)(ffn_start)

            @pl.when(h == H - 1)
            def _():
                for c in range(DOWN_CHUNKS):
                    tall_start(wd_hbm, wd_s, sem_d.at[c], c * FC, FC)

    lax.fori_loop(H - NL, H, functools.partial(head, tail_start), 0)

    hres = x + jnp.sum(acc_s[...], axis=0, keepdims=True)
    hn = _layernorm(hres)
    wr_cp.wait()
    wr = wr_s[...].astype(f32).reshape(1, D)
    gate = jax.nn.sigmoid(jnp.sum(hn * wr, axis=-1, keepdims=True))
    hb = jnp.broadcast_to(hn, (8, D)).astype(bf16)
    done(wg_s, sem_w.at[3])
    g = jnp.dot(hb, wg_s[...], preferred_element_type=f32)
    done(wu_s, sem_w.at[4])
    u = jnp.dot(hb, wu_s[...], preferred_element_type=f32)
    gu = (g * jax.nn.sigmoid(g) * u).astype(bf16)
    y = jnp.zeros((8, D), f32)
    for c in range(DOWN_CHUNKS):
        done(wd_s.at[pl.ds(c * FC, FC)], sem_d.at[c])
        y = y + jnp.dot(gu[:, c * FC:(c + 1) * FC], wd_s[c * FC:(c + 1) * FC, :],
                        preferred_element_type=f32)
    out = hres + (hn + y[:1] * gate)
    o_ref[0] = out.astype(o_ref.dtype)


@jax.jit
def pallas_sequential_preLN__sliding_block_cached__moe_arch_mod__decode_kernel(
    A_x: jax.Array,
    A_k_cache: jax.Array,
    A_v_cache: jax.Array,
    A_wq: jax.Array,
    A_wo: jax.Array,
    B_x: jax.Array,
    B_w_r: jax.Array,
    B_w_gate: jax.Array,
    B_w_up: jax.Array,
    B_w_down: jax.Array,
):
    del B_x
    _, H, Sk, Dh = A_k_cache.shape
    D = A_x.shape[-1]
    W = min(4096, max(256, Sk // 4))
    kt = jnp.transpose(A_k_cache, (0, 1, 3, 2))
    vt = jnp.transpose(A_v_cache, (0, 1, 3, 2))
    like = lambda a: pltpu.VMEM(a.shape, a.dtype)
    return pl.pallas_call(
        _kernel,
        out_shape=jax.ShapeDtypeStruct(A_x.shape, A_x.dtype),
        in_specs=[pl.BlockSpec(memory_space=pl.ANY)] * 9,
        scratch_shapes=[
            like(A_x), like(B_w_r), like(A_wq), like(A_wo),
            like(B_w_gate), like(B_w_up), like(B_w_down),
            pltpu.VMEM((NBUF, Dh, W), A_k_cache.dtype),
            pltpu.VMEM((NBUF, Dh, W), A_v_cache.dtype),
            pltpu.VMEM((H, 8, Dh), jnp.float32),
            pltpu.VMEM((8, W), jnp.float32),
            pltpu.VMEM((8, D), jnp.float32),
            pltpu.SemaphoreType.DMA((6,)),
            pltpu.SemaphoreType.DMA((DOWN_CHUNKS,)),
            pltpu.SemaphoreType.DMA((NBUF,)),
            pltpu.SemaphoreType.DMA((NBUF,)),
        ],
        compiler_params=pltpu.CompilerParams(vmem_limit_bytes=100 * 2**20),
    )(A_x, kt, vt, A_wq, A_wo, B_w_r, B_w_gate, B_w_up, B_w_down)
```

```python
import functools
import jax
import jax.numpy as jnp
from jax import lax
import jax.experimental.pallas as pl
import jax.experimental.pallas.tpu as pltpu

CR, CC = 32, 512
NBUF = 3
DOWN_CHUNKS = 4
EPS = 1e-5


def _layernorm(x):
    m = jnp.mean(x, axis=-1, keepdims=True)
    d = x - m
    v = jnp.mean(d * d, axis=-1, keepdims=True)
    return d / jnp.sqrt(v + EPS)


def _kernel(x_hbm, kt_hbm, vt_hbm, wq_hbm, wo_hbm, wr_hbm, wg_hbm, wu_hbm, wd_hbm,
            o_ref,
            x_s, wr_s, wq_s, wo_s, wg_s, wu_s, wd_s, k_s, v_s, q_s, p_s, acc_s,
            sem_kv, sem_w, sem_d):
    _, H, Dh, Sk = kt_hbm.shape
    W = k_s.shape[-1]
    D = x_hbm.shape[-1]
    F = wg_hbm.shape[-1]
    FC = F // DOWN_CHUNKS
    f32, bf16 = jnp.float32, jnp.bfloat16

    def piece(src, dst, sem, r, c, nc, prio):
        idx = (pl.ds(r, CR), pl.ds(c, nc))
        pltpu.make_async_copy(src.at[idx], dst.at[idx], sem).start(priority=prio)

    def done(dst, sem):
        pltpu.make_async_copy(dst, dst, sem).wait()

    kv_pieces = [(r, c) for r in range(0, Dh, CR) for c in range(0, W, CC)]

    def kv_start(h, pieces):
        sl = h % NBUF
        ks = kt_hbm.at[0, h, :, pl.ds(Sk - W, W)]
        vs = vt_hbm.at[0, h, :, pl.ds(Sk - W, W)]
        for r, c in pieces:
            piece(ks, k_s.at[sl], sem_kv.at[0,sl], r, c, CC, 0)
            piece(vs, v_s.at[sl], sem_kv.at[1,sl], r, c, CC, 1)

    def wide_start(src, dst, sem):
        def body(i, _):
            r = pl.multiple_of(i * CR, CR)
            for n, c in enumerate(range(0, src.shape[1], CC)):
                piece(src, dst, sem, r, c, CC, n % 2)
        lax.fori_loop(0, src.shape[0] // CR, body, None)

    def tall_start(src, dst, sem, r0, n):
        def body(i, _):
            for t in range(2):
                piece(src, dst, sem, pl.multiple_of(r0 + (2 * i + t) * CR, CR), 0, D, t)
        lax.fori_loop(0, n // CR // 2, body, None)

    def ffn_start():
        def body(i, _):
            r = pl.multiple_of(i * CR, CR)
            for c in range(0, F, CC):
                piece(wg_hbm, wg_s, sem_w.at[3], r, c, CC, 0)
                piece(wu_hbm, wu_s, sem_w.at[4], r, c, CC, 1)
        lax.fori_loop(0, D // CR, body, None)

    x_cp = pltpu.make_async_copy(x_hbm, x_s, sem_w.at[1])
    wr_cp = pltpu.make_async_copy(wr_hbm, wr_s, sem_w.at[5])

    x_cp.start()
    wr_cp.start(priority=1)
    wide_start(wq_hbm, wq_s, sem_w.at[0])
    tall_start(wo_hbm, wo_s, sem_w.at[2], 0, H * Dh)

    x_cp.wait()
    x = x_s[0].astype(f32)
    xn = jnp.broadcast_to(_layernorm(x), (8, D)).astype(bf16)
    done(wq_s, sem_w.at[0])
    QC = 2 * Dh
    for c in range(H // 2):
        if c < (NBUF - 1) * 4:
            kv_start(c // 4, kv_pieces[(c % 4) * 12:(c % 4 + 1) * 12])
        q2 = jnp.dot(xn, wq_s[:, c * QC:(c + 1) * QC], preferred_element_type=f32)
        q_s[2 * c] = q2[:, :Dh]
        q_s[2 * c + 1] = q2[:, Dh:]
    acc_s[...] = jnp.zeros_like(acc_s)
    done(wo_s, sem_w.at[2])

    scale = Dh ** -0.5

    def head(start, h, carry):
        slot = h % NBUF
        done(k_s.at[slot], sem_kv.at[0,slot])
        s = jnp.dot(q_s[h].astype(bf16), k_s[slot], preferred_element_type=f32) * scale
        m = jnp.max(s, axis=-1, keepdims=True)
        e = jnp.exp(s - m)
        l = jnp.sum(e, axis=-1, keepdims=True)
        p_s[...] = e
        inv = 1.0 / l
        done(v_s.at[slot], sem_kv.at[1,slot])
        row0 = pl.multiple_of(h * Dh, 64)
        acc = acc_s[...]
        for r in range(Dh // 16):
            start(h, r)
            a0 = jnp.zeros((8, 128), f32)
            a1 = jnp.zeros((8, 128), f32)
            for j in range(W // 128):
                vv = v_s[slot, r * 16:(r + 1) * 16, j * 128:(j + 1) * 128].astype(f32)
                pp = p_s[:, j * 128:(j + 1) * 128]
                a0 = a0 + vv[:8] * pp
                a1 = a1 + vv[8:] * pp
            o0 = jnp.sum(a0, axis=-1, keepdims=True) * inv
            o1 = jnp.sum(a1, axis=-1, keepdims=True) * inv
            ww = wo_s[pl.ds(row0 + r * 16, 16), :].astype(f32)
            acc = acc + ww[:8] * o0 + ww[8:] * o1
        acc_s[...] = acc
        return carry

    NL = NBUF - 1
    PR = len(kv_pieces) // (Dh // 16)
    lax.fori_loop(0, H - NL, functools.partial(
        head, lambda h, r: kv_start(h + NL, kv_pieces[r * PR:(r + 1) * PR])), 0)

    def tail_start(h, r):
        if r == 0:
            pl.when(h == H - NL)(ffn_start)

            @pl.when(h == H - 1)
            def _():
                for c in range(DOWN_CHUNKS):
                    tall_start(wd_hbm, wd_s, sem_d.at[c], c * FC, FC)

    lax.fori_loop(H - NL, H, functools.partial(head, tail_start), 0)

    hres = x + jnp.sum(acc_s[...], axis=0, keepdims=True)
    hn = _layernorm(hres)
    wr_cp.wait()
    wr = wr_s[...].astype(f32).reshape(1, D)
    gate = jax.nn.sigmoid(jnp.sum(hn * wr, axis=-1, keepdims=True))
    hb = jnp.broadcast_to(hn, (8, D)).astype(bf16)
    done(wg_s, sem_w.at[3])
    g = jnp.dot(hb, wg_s[...], preferred_element_type=f32)
    done(wu_s, sem_w.at[4])
    u = jnp.dot(hb, wu_s[...], preferred_element_type=f32)
    gu = (g * jax.nn.sigmoid(g) * u).astype(bf16)
    y = jnp.zeros((8, D), f32)
    for c in range(DOWN_CHUNKS):
        done(wd_s.at[pl.ds(c * FC, FC)], sem_d.at[c])
        y = y + jnp.dot(gu[:, c * FC:(c + 1) * FC], wd_s[c * FC:(c + 1) * FC, :],
                        preferred_element_type=f32)
    out = hres + (hn + y[:1] * gate)
    o_ref[0] = out.astype(o_ref.dtype)


@jax.jit
def pallas_sequential_preLN__sliding_block_cached__moe_arch_mod__decode_kernel(
    A_x: jax.Array,
    A_k_cache: jax.Array,
    A_v_cache: jax.Array,
    A_wq: jax.Array,
    A_wo: jax.Array,
    B_x: jax.Array,
    B_w_r: jax.Array,
    B_w_gate: jax.Array,
    B_w_up: jax.Array,
    B_w_down: jax.Array,
):
    del B_x
    _, H, Sk, Dh = A_k_cache.shape
    D = A_x.shape[-1]
    W = min(4096, max(256, Sk // 4))
    kt = jnp.transpose(A_k_cache, (0, 1, 3, 2))
    vt = jnp.transpose(A_v_cache, (0, 1, 3, 2))
    like = lambda a: pltpu.VMEM(a.shape, a.dtype)
    return pl.pallas_call(
        _kernel,
        out_shape=jax.ShapeDtypeStruct(A_x.shape, A_x.dtype),
        in_specs=[pl.BlockSpec(memory_space=pl.ANY)] * 9,
        scratch_shapes=[
            like(A_x), like(B_w_r), like(A_wq), like(A_wo),
            like(B_w_gate), like(B_w_up), like(B_w_down),
            pltpu.VMEM((NBUF, Dh, W), A_k_cache.dtype),
            pltpu.VMEM((NBUF, Dh, W), A_v_cache.dtype),
            pltpu.VMEM((H, 8, Dh), jnp.float32),
            pltpu.VMEM((8, W), jnp.float32),
            pltpu.VMEM((8, D), jnp.float32),
            pltpu.SemaphoreType.DMA((2,NBUF)),pltpu.SemaphoreType.DMA((6,)),
            pltpu.SemaphoreType.DMA((DOWN_CHUNKS,)),
        ],
        compiler_params=pltpu.CompilerParams(vmem_limit_bytes=100 * 2**20),
    )(A_x, kt, vt, A_wq, A_wo, B_w_r, B_w_gate, B_w_up, B_w_down)
```
